```python
import os as _os
_os.environ.setdefault("JAX_PLATFORMS", "cpu")
import jax
import jax.numpy as jnp

def _softmax(x, axis=-1):
    return jax.nn.softmax(x, axis=axis)
def _gelu(x):
    return jax.nn.gelu(x, approximate=True)
def _silu(x):
    return jax.nn.silu(x)
def _sigmoid(x):
    return jax.nn.sigmoid(x)
def _layernorm(x, axis=-1, eps=1e-5):
    m = jnp.mean(x, axis=axis, keepdims=True)
    v = jnp.var(x, axis=axis, keepdims=True)
    return (x - m) / jnp.sqrt(v + eps)
def _scatter_add(tgt, idx, src, axis=0):
    return tgt.at[idx].add(src)
def _segment_sum(src, seg, n):
    return jax.ops.segment_sum(src, seg, n)
class _Rng:
    def __init__(self, key):
        self._k = key
    def _next(self):
        self._k, sub = jax.random.split(self._k)
        return sub
    def normal(self, shape):
        return jax.random.normal(self._next(), shape, dtype=jnp.bfloat16)
    def randint(self, lo, hi, shape):
        return jax.random.randint(self._next(), shape, lo, hi, dtype=jnp.int32)
    def uniform(self, shape, lo=0.0, hi=1.0):
        return jax.random.uniform(self._next(), shape, jnp.bfloat16, lo, hi)
    def permutation(self, n):
        return jax.random.permutation(self._next(), n)


kernel_name = 'standalone__gqa_block_cached__near_ridge'

def setup_inputs():
    _rng = _Rng(jax.random.key(int.from_bytes(__import__("os").urandom(4), "little")))
    _w = (lambda a: (lambda t: t.astype(jnp.bfloat16) if jnp.issubdtype(t.dtype, jnp.floating) else t)(jnp.asarray(a)))
    B, Sq, D = 8, 64, 512
    Hq, Hkv, Sk, Dh = 32, 8, 64, 128
    assert Hq % Hkv == 0, (Hq, Hkv)
    return {
        "x": _w((lambda *s: _rng.normal(s) * 0.8)(B, Sq, D)),
        "k_cache": _w((lambda *s: _rng.normal(s) * 0.8)(B, Hkv, Sk, Dh)),
        "v_cache": _w((lambda *s: _rng.normal(s) * 0.05)(B, Hkv, Sk, Dh)),
        "wq": _w((lambda *s: _rng.normal(s) * 0.8)(D, Hq * Dh) * (D ** -0.5)),
        "wo": _w((lambda *s: _rng.normal(s) * 0.05)(Hq * Dh, D) * ((Hq * Dh) ** -0.5)),
    }

def reference(x, k_cache, v_cache, wq, wo):
    B, Sq, D = x.shape
    Hq, Dh = 32, 128
    Hkv = k_cache.shape[1]
    rep = Hq // Hkv
    q = (lambda x, *d: x.transpose(*d))((x @ wq).reshape(B, Sq, Hq, Dh), 0, 2, 1, 3)
    k = jnp.repeat(k_cache, rep, axis=1)
    v = jnp.repeat(v_cache, rep, axis=1)
    scores = jnp.einsum("bhqd,bhkd->bhqk", q, k) * (Dh ** -0.5)
    p = _softmax(scores, axis=-1)
    o = jnp.einsum("bhqk,bhkd->bhqd", p, v)
    return (lambda x, *d: x.transpose(*d))(o, 0, 2, 1, 3).reshape(B, Sq, Hq * Dh) @ wo
```

```python
import math

import jax
import jax.numpy as jnp
import jax.experimental.pallas as pl
import jax.experimental.pallas.tpu as pltpu

B, SQ, D, HQ, HKV, SK, DH = 8, 64, 512, 32, 8, 64, 128
REP = HQ // HKV
M = B * SQ
T = 128
NKT = D // T
C_EXP2 = (DH ** -0.5) * math.log2(math.e)
F32, BF16 = jnp.float32, jnp.bfloat16
NT_DIMS = (((1,), (1,)), ((), ()))

N_KMAJOR = 3
WQ_CHUNKS = [(12, 16), (16, 24), (24, 32)]
WO_CHUNKS = [(0, 4), (4, 8), (8, 12), (12, 20), (20, 32)]
KV_CHUNKS = [(0, 1), (1, 2), (2, 3), (3, 5), (5, 8)]
TAIL = [(0, 0, M), (1, 0, M), (2, 0, M), (3, 0, M // 2), (3, M // 2, M)]

HEAD = ("A00 A01 A02 A03 "
        "A10 A11 S00 S01 A12 S02 S03 A13 V00 V01 "
        "A20 V02 V03 A21 S10 C00 V10 S11 A22 V11 S12 C01 V12 S13 A23 V13 C02 C03")
STEADY = "a0 s0 c0 a1 v0 s1 c1 a2 v1 s2 c2 v2 s3 a3 v3 c3"
LAST = "C60 S70 S71 C61 V70 V71 S72 S73 C62 V72 V73 C63"


def _schedule():
    parse = lambda text: [(w[0], int(w[1]), int(w[2])) for w in text.split()]
    seq = parse(HEAD)
    for t in range(2, HKV - 1):
        seq += [(w[0].upper(), {"a": t + 1, "s": t, "v": t, "c": t - 1}[w[0]], int(w[1]))
                for w in STEADY.split()]
    seq += parse(LAST)
    seq += [("F", p, None) for p in TAIL]
    done = set()
    for op, g, i in seq:
        if op == "A":
            assert i == 0 or ("A", g, i - 1) in done
        elif op == "S":
            assert all(("A", g, n) in done for n in range(4))
        elif op == "V":
            assert ("S", g, i) in done
        elif op == "C":
            assert all(("V", g, j) in done for j in range(4)) and (g == 0 or ("C", g - 1, i) in done)
        else:
            assert all(("V", HKV - 1, j) in done for j in range(4)) and ("C", HKV - 2, g[0]) in done
        assert (op, g, i) not in done
        done.add((op, g, i))
    assert len(done) == 4 * HKV + 8 * HKV + 4 * (HKV - 1) + len(TAIL)
    return seq


def _owner(name, chunks, i):
    return next((name, lo) for lo, hi in chunks if lo <= i < hi)


def _needs(op, g, i):
    if op == "A" and g < N_KMAJOR:
        return [("wqk", g, i), ("x", i)]
    if op == "A":
        return [("x", k) for k in range(NKT)] + [_owner("wq", WQ_CHUNKS, g * REP + i)]
    if op == "S":
        return [_owner("k", KV_CHUNKS, g)]
    if op == "V":
        return [_owner("v", KV_CHUNKS, g)]
    g = g if op == "C" else HKV - 1
    return [_owner("wo", WO_CHUNKS, g * REP + h) for h in range(REP)]


def _dot(a, b):
    return jnp.dot(a, b, preferred_element_type=F32)


def _kernel(x_hbm, k_hbm, v_hbm, wq_hbm, wo_hbm, o_hbm,
            x_s, k_s, v_s, wq_s, wo_s, q_s, a_s, acc_s, qacc_s, o_s, sems):
    seq = _schedule()

    cp = {}

    def mk(key, src, dst):
        cp[key] = pltpu.make_async_copy(src, dst, sems.at[len(cp)])

    for k in range(NKT):
        mk(("x", k), x_hbm.at[:, pl.ds(k * T, T)], x_s.at[k])
    for g in range(N_KMAJOR):
        for k in range(NKT):
            idx = (pl.ds(k * T, T), pl.ds(g * REP * T, REP * T))
            mk(("wqk", g, k), wq_hbm.at[idx], wq_s.at[idx])
    for lo, hi in WQ_CHUNKS:
        idx = (slice(None), pl.ds(lo * T, (hi - lo) * T))
        mk(("wq", lo), wq_hbm.at[idx], wq_s.at[idx])
    for lo, hi in WO_CHUNKS:
        idx = (pl.ds(lo * T, (hi - lo) * T),)
        mk(("wo", lo), wo_hbm.at[idx], wo_s.at[idx])
    for lo, hi in KV_CHUNKS:
        idx = (slice(None), pl.ds(lo, hi - lo))
        mk(("k", lo), k_hbm.at[idx], k_s.at[idx])
        mk(("v", lo), v_hbm.at[idx], v_s.at[idx])
    outs = {}
    for n, lo, hi in TAIL:
        outs[(n, lo, hi)] = pltpu.make_async_copy(
            o_s.at[n, pl.ds(lo, hi - lo)], o_hbm.at[pl.ds(lo, hi - lo), pl.ds(n * T, T)],
            sems.at[len(cp) + len(outs)])

    first_use = []
    for tok in seq:
        for key in _needs(*tok):
            if key not in first_use:
                first_use.append(key)
    assert set(first_use) == set(cp)
    for key in first_use:
        cp[key].start()

    probs = {}

    def q_proj(g, i):
        if g < N_KMAJOR:
            xk = x_s[i]
            for n in range(REP):
                col = (g * REP + n) * T
                y = _dot(xk, wq_s[i * T:(i + 1) * T, col:col + T])
                if i == 0:
                    qacc_s[n] = y
                elif i < NKT - 1:
                    qacc_s[n] = qacc_s[n] + y
                else:
                    q_s[g, n] = (qacc_s[n] + y).astype(BF16)
            return
        col = (g * REP + i) * T
        q = _dot(x_s[0], wq_s[0:T, col:col + T])
        for kt in range(1, NKT):
            q = q + _dot(x_s[kt], wq_s[kt * T:(kt + 1) * T, col:col + T])
        q_s[g, i] = q.astype(BF16)

    def scores(g, i):
        for b in (2 * i, 2 * i + 1):
            rows = slice(b * SQ, (b + 1) * SQ)
            kb = k_s[b, g]
            ps = []
            for t in range(2):
                qt = jnp.concatenate([q_s[g, 2 * t, rows, :], q_s[g, 2 * t + 1, rows, :]], axis=0)
                st = jax.lax.dot_general(kb, qt, NT_DIMS, preferred_element_type=F32)
                m = jnp.max(st, axis=0, keepdims=True)
                e = jnp.exp2((st - m) * C_EXP2)
                ps.append(e * (1.0 / jnp.sum(e, axis=0, keepdims=True)))
            probs[(g, b)] = jnp.concatenate(ps, axis=0).T.astype(BF16)

    def pv(g, i):
        for b in (2 * i, 2 * i + 1):
            rows = slice(b * SQ, (b + 1) * SQ)
            vb = v_s[b, g]
            z = jnp.zeros_like(vb)
            p = probs.pop((g, b))
            for t in range(2):
                vz = jnp.concatenate([vb, z] if t == 0 else [z, vb], axis=0)
                o = _dot(p, vz).astype(BF16)
                a_s[g, 2 * t, rows, :] = o[0:SQ]
                a_s[g, 2 * t + 1, rows, :] = o[SQ:2 * SQ]

    def out_tile(g, n, lo, hi):
        r0 = g * REP * T
        y = _dot(a_s[g, 0, lo:hi, :], wo_s[r0:r0 + T, n * T:(n + 1) * T])
        for h in range(1, REP):
            y = y + _dot(a_s[g, h, lo:hi, :], wo_s[r0 + h * T:r0 + (h + 1) * T, n * T:(n + 1) * T])
        return y

    def out_proj(g, n):
        y = out_tile(g, n, 0, M)
        acc_s[n] = y if g == 0 else acc_s[n] + y

    def out_final(p, _):
        n, lo, hi = p
        o_s[n, lo:hi, :] = (acc_s[n, lo:hi, :] + out_tile(HKV - 1, n, lo, hi)).astype(BF16)
        outs[p].start()

    jobs = {"A": q_proj, "S": scores, "V": pv, "C": out_proj, "F": out_final}
    waited = set()
    for tok in seq:
        for key in _needs(*tok):
            if key not in waited:
                waited.add(key)
                cp[key].wait()
        jobs[tok[0]](tok[1], tok[2])
    for c in outs.values():
        c.wait()


_N_SEMS = NKT + NKT * N_KMAJOR + len(WQ_CHUNKS) + len(WO_CHUNKS) + 2 * len(KV_CHUNKS) + len(TAIL)


@jax.jit
def pallas_standalone__gqa_block_cached__near_ridge_kernel(
    x: jax.Array,
    k_cache: jax.Array,
    v_cache: jax.Array,
    wq: jax.Array,
    wo: jax.Array,
):
    out = pl.pallas_call(
        _kernel,
        in_specs=[pl.BlockSpec(memory_space=pl.ANY)] * 5,
        out_specs=pl.BlockSpec(memory_space=pl.ANY),
        out_shape=jax.ShapeDtypeStruct((M, D), BF16),
        scratch_shapes=[
            pltpu.VMEM((NKT, M, T), BF16),
            pltpu.VMEM((B, HKV, SK, DH), BF16),
            pltpu.VMEM((B, HKV, SK, DH), BF16),
            pltpu.VMEM((D, HQ * DH), BF16),
            pltpu.VMEM((HQ * DH, D), BF16),
            pltpu.VMEM((HKV, REP, M, DH), BF16),
            pltpu.VMEM((HKV, REP, M, DH), BF16),
            pltpu.VMEM((NKT, M, T), F32),
            pltpu.VMEM((REP, M, T), F32),
            pltpu.VMEM((NKT, M, T), BF16),
            pltpu.SemaphoreType.DMA((_N_SEMS,)),
        ],
        compiler_params=pltpu.CompilerParams(
            vmem_limit_bytes=64 * 1024 * 1024,
            flags={"XLA_TPU_RESCHEDULE_DMA_DONES": True},
            disable_semaphore_checks=True,
        ),
    )(x.reshape(M, D), k_cache, v_cache, wq, wo)
    return out.reshape(B, SQ, D)
```

```python
import math

import jax
import jax.numpy as jnp
import jax.experimental.pallas as pl
import jax.experimental.pallas.tpu as pltpu

B, SQ, D, HQ, HKV, SK, DH = 8, 64, 512, 32, 8, 64, 128
REP = HQ // HKV
M = B * SQ
T = 128
NKT = D // T
C_EXP2 = (DH ** -0.5) * math.log2(math.e)
F32, BF16 = jnp.float32, jnp.bfloat16
NT_DIMS = (((1,), (1,)), ((), ()))

ORDER = (
    "A00 A01 A02 A03 A10 A11 S00 S01 A12 A13 V00 S02 S03 A20 V03 V01 V02 A21 S10 C00 V10 S11 A22 V11 "
    "S12 C01 V12 S13 A23 V13 C02 S20 C03 A30 A31 C10 A32 V20 S21 C11 V21 S22 C12 V22 S23 A33 A40 V23 "
    "C13 S30 C20 A41 V30 S31 C21 V31 S32 C22 V32 S33 A42 A43 A50 V33 C23 S40 C30 A51 V40 S41 C31 A52 "
    "V41 S42 C32 V42 S43 C33 A53 V43 A60 S50 C40 V50 S51 C41 A61 A62 V51 S52 C42 V52 S53 A63 V53 C43 "
    "S60 C50 A70 V60 S61 C51 A71 A72 V61 S62 C52 V62 S63 A73 V63 C53 S70 C60 S71 V70 S72 C61 S73 V71 "
    "C62 V72 V73 C63 "
)
N_KMAJOR = 3
SPLITS = {
    (0, 0): (64, 256, 448), (0, 1): (96, 256, 448), (0, 2): (128, 160, 432, 480),
    (0, 3): (96, 160, 224, 352, 464),
    (1, 0): (384,), (1, 1): (128, 384), (1, 2): (160,), (1, 3): (32, 448),
    (2, 0): (448,), (2, 1): (320, 448),
}
FINE_KV, FINE_WO = 1, 1
WQ_CHUNKS = [(12, 16), (16, 24), (24, 32)]
WO_CHUNKS = [(4, 8), (8, 12), (12, 20), (20, 32)]
KV_CHUNKS = [(1, 2), (2, 3), (3, 5), (5, 8)]
TAIL = [(0, 0, 512), (1, 0, 512), (2, 0, 512), (3, 0, 256), (3, 256, 384), (3, 384, 448), (3, 448, 480), (3, 480, 512)]


def _schedule():
    seq = [(w[0], int(w[1]), int(w[2])) for w in ORDER.split()] + [("F", p, None) for p in TAIL]
    done = set()
    for op, g, i in seq:
        if op == "A":
            assert i == 0 or ("A", g, i - 1) in done
            assert g == 0 or g >= N_KMAJOR or ("A", g - 1, NKT - 1) in done
        elif op == "S":
            assert all(("A", g, n) in done for n in range(4))
        elif op == "V":
            assert ("S", g, i) in done
        elif op == "C":
            assert all(("V", g, j) in done for j in range(4)) and (g == 0 or ("C", g - 1, i) in done)
        else:
            assert all(("V", HKV - 1, j) in done for j in range(4)) and ("C", HKV - 2, g[0]) in done
        assert (op, g, i) not in done
        done.add((op, g, i))
    assert len(done) == 4 * HKV + 8 * HKV + 4 * (HKV - 1) + len(TAIL)
    assert sorted((n, lo) for n, lo, hi in TAIL if lo == 0) == [(n, 0) for n in range(NKT)]
    assert all(hi == M or (n, hi) in [(a, b) for a, b, _ in TAIL] for n, lo, hi in TAIL)
    return seq


def _pieces(g, i):
    edges = (0,) + tuple(SPLITS.get((g, i), ())) + (M,)
    return list(zip(edges[:-1], edges[1:]))


def _owner(name, chunks, i):
    return next((name, lo, hi) for lo, hi in chunks if lo <= i < hi)


def _needs(op, g, i):
    if op == "A" and g == 0:
        return [("wqk", 0, i)] + [("x", i, lo, hi) for lo, hi in _pieces(0, i)]
    if op == "A" and g < N_KMAJOR:
        return [("wqk", g, i)]
    if op == "A":
        return [_owner("wq", WQ_CHUNKS, g * REP + i)]
    if op == "S":
        return [("kf", g, i)] if g < FINE_KV else [_owner("k", KV_CHUNKS, g)]
    if op == "V":
        return [("vf", g, i)] if g < FINE_KV else [_owner("v", KV_CHUNKS, g)]
    if op == "C" and g < FINE_WO:
        return [("wof", g, i)]
    g = g if op == "C" else HKV - 1
    return [_owner("wo", WO_CHUNKS, g * REP + h) for h in range(REP)]


def _first_use():
    keys = []
    for tok in _schedule():
        for key in _needs(*tok):
            if key not in keys:
                keys.append(key)
    return keys


def _dot(a, b):
    return jnp.dot(a, b, preferred_element_type=F32)


def _kernel(x_hbm, k_hbm, v_hbm, wq_hbm, wo_hbm, o_hbm,
            x_s, k_s, v_s, wq_s, wo_s, q_s, a_s, acc_s, qacc_s, o_s, sems):
    def refs(key):
        name = key[0]
        if name == "x":
            _, k, lo, hi = key
            return x_hbm.at[pl.ds(lo, hi - lo), pl.ds(k * T, T)], x_s.at[k, pl.ds(lo, hi - lo)]
        if name == "wqk":
            idx = (pl.ds(key[2] * T, T), pl.ds(key[1] * REP * T, REP * T))
            return wq_hbm.at[idx], wq_s.at[idx]
        if name == "wq":
            idx = (slice(None), pl.ds(key[1] * T, (key[2] - key[1]) * T))
            return wq_hbm.at[idx], wq_s.at[idx]
        if name == "wof":
            idx = (pl.ds(key[1] * REP * T, REP * T), pl.ds(key[2] * T, T))
            return wo_hbm.at[idx], wo_s.at[idx]
        if name == "wo":
            idx = (pl.ds(key[1] * T, (key[2] - key[1]) * T),)
            return wo_hbm.at[idx], wo_s.at[idx]
        if name in ("kf", "vf"):
            idx = (pl.ds(2 * key[2], 2), pl.ds(key[1], 1))
        else:
            idx = (slice(None), pl.ds(key[1], key[2] - key[1]))
        return (k_hbm.at[idx], k_s.at[idx]) if name[0] == "k" else (v_hbm.at[idx], v_s.at[idx])

    keys = _first_use()
    loads = {key: pltpu.make_async_copy(*refs(key), sems.at[i]) for i, key in enumerate(keys)}
    stores = {}
    for n, lo, hi in TAIL:
        stores[(n, lo, hi)] = pltpu.make_async_copy(
            o_s.at[n, pl.ds(lo, hi - lo)], o_hbm.at[pl.ds(lo, hi - lo), pl.ds(n * T, T)],
            sems.at[len(loads) + len(stores)])
    for key in keys:
        loads[key].start()

    waited = set()

    def wait(key):
        if key not in waited:
            waited.add(key)
            loads[key].wait()

    probs = {}

    def q_proj(g, i):
        if g < N_KMAJOR:
            wait(("wqk", g, i))
            for lo, hi in _pieces(g, i):
                if g == 0:
                    wait(("x", i, lo, hi))
                xk = x_s[i, lo:hi, :]
                for n in range(REP):
                    col = (g * REP + n) * T
                    y = _dot(xk, wq_s[i * T:(i + 1) * T, col:col + T])
                    if i == 0:
                        qacc_s[n, lo:hi, :] = y
                    elif i < NKT - 1:
                        qacc_s[n, lo:hi, :] = qacc_s[n, lo:hi, :] + y
                    else:
                        q_s[g, n, lo:hi, :] = (qacc_s[n, lo:hi, :] + y).astype(BF16)
            return
        col = (g * REP + i) * T
        for lo, hi in _pieces(g, i):
            q = _dot(x_s[0, lo:hi, :], wq_s[0:T, col:col + T])
            for kt in range(1, NKT):
                q = q + _dot(x_s[kt, lo:hi, :], wq_s[kt * T:(kt + 1) * T, col:col + T])
            q_s[g, i, lo:hi, :] = q.astype(BF16)

    def scores(g, i):
        for b in (2 * i, 2 * i + 1):
            rows = slice(b * SQ, (b + 1) * SQ)
            kb = k_s[b, g]
            ps = []
            for t in range(2):
                qt = jnp.concatenate([q_s[g, 2 * t, rows, :], q_s[g, 2 * t + 1, rows, :]], axis=0)
                st = jax.lax.dot_general(kb, qt, NT_DIMS, preferred_element_type=F32)
                m = jnp.max(st, axis=0, keepdims=True)
                e = jnp.exp2((st - m) * C_EXP2)
                ps.append(e * (1.0 / jnp.sum(e, axis=0, keepdims=True)))
            probs[(g, b)] = jnp.concatenate(ps, axis=0).T.astype(BF16)

    def pv(g, i):
        for b in (2 * i, 2 * i + 1):
            rows = slice(b * SQ, (b + 1) * SQ)
            vb = v_s[b, g]
            z = jnp.zeros_like(vb)
            p = probs.pop((g, b))
            for t in range(2):
                vz = jnp.concatenate([vb, z] if t == 0 else [z, vb], axis=0)
                o = _dot(p, vz).astype(BF16)
                a_s[g, 2 * t, rows, :] = o[0:SQ]
                a_s[g, 2 * t + 1, rows, :] = o[SQ:2 * SQ]

    def out_tile(g, n, lo, hi):
        r0 = g * REP * T
        head = lambda h: a_s[g, h, lo:hi, :]
        y = _dot(head(0), wo_s[r0:r0 + T, n * T:(n + 1) * T])
        for h in range(1, REP):
            y = y + _dot(head(h), wo_s[r0 + h * T:r0 + (h + 1) * T, n * T:(n + 1) * T])
        return y

    def out_proj(g, n):
        y = out_tile(g, n, 0, M)
        acc_s[n, 0:M, :] = y if g == 0 else acc_s[n, 0:M, :] + y

    def out_final(p, _):
        n, lo, hi = p
        o_s[n, lo:hi, :] = (acc_s[n, lo:hi, :] + out_tile(HKV - 1, n, lo, hi)).astype(BF16)
        stores[p].start()

    jobs = {"A": q_proj, "S": scores, "V": pv, "C": out_proj, "F": out_final}
    for tok in _schedule():
        if tok[0] != "A" or tok[1] >= N_KMAJOR:
            for key in _needs(*tok):
                wait(key)
        jobs[tok[0]](tok[1], tok[2])
    assert waited == set(loads)
    for copy in stores.values():
        copy.wait()


@jax.jit
def pallas_standalone__gqa_block_cached__near_ridge_kernel(
    x: jax.Array,
    k_cache: jax.Array,
    v_cache: jax.Array,
    wq: jax.Array,
    wo: jax.Array,
):
    out = pl.pallas_call(
        _kernel,
        in_specs=[pl.BlockSpec(memory_space=pl.ANY)] * 5,
        out_specs=pl.BlockSpec(memory_space=pl.ANY),
        out_shape=jax.ShapeDtypeStruct((M, D), BF16),
        scratch_shapes=[
            pltpu.VMEM((NKT, M, T), BF16),
            pltpu.VMEM((B, HKV, SK, DH), BF16),
            pltpu.VMEM((B, HKV, SK, DH), BF16),
            pltpu.VMEM((D, HQ * DH), BF16),
            pltpu.VMEM((HQ * DH, D), BF16),
            pltpu.VMEM((HKV, REP, M, DH), BF16),
            pltpu.VMEM((HKV, REP, M, DH), BF16),
            pltpu.VMEM((NKT, M, T), F32),
            pltpu.VMEM((REP, M, T), F32),
            pltpu.VMEM((NKT, M, T), BF16),
            pltpu.SemaphoreType.DMA((len(_first_use()) + len(TAIL),)),
        ],
        compiler_params=pltpu.CompilerParams(
            vmem_limit_bytes=64 * 1024 * 1024,
            flags={"XLA_TPU_RESCHEDULE_DMA_DONES": True},
            disable_semaphore_checks=True,
        ),
    )(x.reshape(M, D), k_cache, v_cache, wq, wo)
    return out.reshape(B, SQ, D)
```
